```python
import os as _os
_os.environ.setdefault("JAX_PLATFORMS", "cpu")
import jax
import jax.numpy as jnp

def _softmax(x, axis=-1):
    return jax.nn.softmax(x, axis=axis)
def _gelu(x):
    return jax.nn.gelu(x, approximate=True)
def _silu(x):
    return jax.nn.silu(x)
def _sigmoid(x):
    return jax.nn.sigmoid(x)
def _layernorm(x, axis=-1, eps=1e-5):
    m = jnp.mean(x, axis=axis, keepdims=True)
    v = jnp.var(x, axis=axis, keepdims=True)
    return (x - m) / jnp.sqrt(v + eps)
def _scatter_add(tgt, idx, src, axis=0):
    return tgt.at[idx].add(src)
def _segment_sum(src, seg, n):
    return jax.ops.segment_sum(src, seg, n)
class _Rng:
    def __init__(self, key):
        self._k = key
    def _next(self):
        self._k, sub = jax.random.split(self._k)
        return sub
    def normal(self, shape):
        return jax.random.normal(self._next(), shape, dtype=jnp.bfloat16)
    def randint(self, lo, hi, shape):
        return jax.random.randint(self._next(), shape, lo, hi, dtype=jnp.int32)
    def uniform(self, shape, lo=0.0, hi=1.0):
        return jax.random.uniform(self._next(), shape, jnp.bfloat16, lo, hi)
    def permutation(self, n):
        return jax.random.permutation(self._next(), n)


kernel_name = 'standalone__gqa_softmax__near_ridge'

def setup_inputs():
    _rng = _Rng(jax.random.key(int.from_bytes(__import__("os").urandom(4), "little")))
    _w = (lambda a: (lambda t: t.astype(jnp.bfloat16) if jnp.issubdtype(t.dtype, jnp.floating) else t)(jnp.asarray(a)))
    B, Hq, Hkv, Sq, Sk, D = 8, 16, 8, 512, 512, 256
    return {
        "q": _w((lambda *s: _rng.normal(s) * 0.4)(B, Hq, Sq, D)),
        "k": _w((lambda *s: _rng.normal(s) * 0.4)(B, Hkv, Sk, D)),
        "v": _w((lambda *s: _rng.normal(s) * 0.05)(B, Hkv, Sk, D)),
    }

def reference(q, k, v):
    B, Hq, Sq, D = q.shape
    Hkv = k.shape[1]
    rep = Hq // Hkv
    k = jnp.repeat(k, rep, axis=1)
    v = jnp.repeat(v, rep, axis=1)
    scale = D ** -0.5
    scores = jnp.einsum("bhqd,bhkd->bhqk", q, k) * scale
    p = _softmax(scores, axis=-1)
    return jnp.einsum("bhqk,bhkd->bhqd", p, v)
```

```python
import functools
import math

import jax
import jax.numpy as jnp
import jax.experimental.pallas as pl
import jax.experimental.pallas.tpu as pltpu


def _attn_kernel(q_ref, k_ref, v_ref, o_ref, *, scale):
    q = q_ref[...]
    k = k_ref[...]
    v = v_ref[...]
    s = jax.lax.dot_general(q, k, (((1,), (1,)), ((), ())),
                            preferred_element_type=jnp.float32)
    m = jnp.max(s, axis=-1, keepdims=True)
    p = jnp.exp2((s - m) * (scale * math.log2(math.e)))
    l = jnp.sum(p, axis=-1, keepdims=True)
    o = jnp.dot(p.astype(jnp.bfloat16), v, preferred_element_type=jnp.float32)
    o_ref[...] = (o * (1.0 / l)).astype(o_ref.dtype)


@jax.jit
def pallas_standalone__gqa_softmax__near_ridge_kernel(
    q: jax.Array,
    k: jax.Array,
    v: jax.Array,
):
    B, Hq, Sq, D = q.shape
    Hkv, Sk = k.shape[1], k.shape[2]
    rep = Hq // Hkv
    G = B * Hkv
    M = rep * Sq
    q3 = q.reshape(G, M, D)
    k3 = k.reshape(G, Sk, D)
    v3 = v.reshape(G, Sk, D)
    scale = D ** -0.5
    out = pl.pallas_call(
        functools.partial(_attn_kernel, scale=scale),
        grid=(G,),
        in_specs=[
            pl.BlockSpec((None, M, D), lambda g: (g, 0, 0)),
            pl.BlockSpec((None, Sk, D), lambda g: (g, 0, 0)),
            pl.BlockSpec((None, Sk, D), lambda g: (g, 0, 0)),
        ],
        out_specs=pl.BlockSpec((None, M, D), lambda g: (g, 0, 0)),
        out_shape=jax.ShapeDtypeStruct((G, M, D), q.dtype),
        compiler_params=pltpu.CompilerParams(
            dimension_semantics=("parallel",),
            vmem_limit_bytes=64 * 1024 * 1024,
        ),
    )(q3, k3, v3)
    return out.reshape(B, Hq, Sq, D)
```

```python
import functools
import math

import jax, jax.numpy as jnp
from jax import lax
import jax.experimental.pallas as pl
import jax.experimental.pallas.tpu as pltpu

def _recip(l, recip):
    if recip == "approx":
        return pl.reciprocal(l, approx=True)
    elif recip == "nr":
        r = pl.reciprocal(l, approx=True)
        return r * (2.0 - l * r)
    return 1.0 / l

def qk(q, k):
    return jax.lax.dot_general(q, k, (((1,), (1,)), ((), ())), preferred_element_type=jnp.float32)

def softmax(s, scale, recip):
    m = jnp.max(s, axis=-1, keepdims=True)
    p = jnp.exp2((s - m) * (scale * math.log2(math.e)))
    l = jnp.sum(p, axis=-1, keepdims=True)
    p = p * _recip(l, recip)
    return p.astype(jnp.bfloat16)

def pipeline(units, getq, getk, getv, put, scale, recip, before_qk=None, before_pv=None, after_mxu=None):
    n = len(units)
    def do_qk(u):
        if before_qk: before_qk(u)
        h, r0, r1 = units[u]
        s = qk(getq(h, r0, r1), getk(h))
        if after_mxu: after_mxu()
        return s
    s_next = do_qk(0)
    for u in range(n):
        s = s_next
        if u + 1 < n:
            s_next = do_qk(u + 1)
        p = softmax(s, scale, recip)
        if before_pv: before_pv(u)
        h, r0, r1 = units[u]
        o = jnp.dot(p, getv(h), preferred_element_type=jnp.float32)
        if after_mxu: after_mxu()
        put(u, h, r0, r1, o)

def _kernel(q_hbm, k_hbm, v_hbm, o_hbm, qb, kb, vb, ob, rsem, isem, osem, *,
            scale, nh, G, M, ramp, recip, ns, ur, ur0, split0, tail, lead):
    ng = G // nh
    groups = []
    need_q = {}; need_k = {}; need_v = {}
    def add(gidx, kind, h0, n, r0=0, r1=M):
        hs = pl.ds(h0, n)
        if kind == "q":
            if r0 == 0 and r1 == M:
                groups[gidx].append((q_hbm.at[hs], qb.at[hs]))
            else:
                assert n == 1
                groups[gidx].append((q_hbm.at[h0, r0:r1], qb.at[h0, r0:r1]))
            for h in range(h0, h0 + n):
                for r in range(r0, r1, 8): need_q[(h, r)] = gidx
        elif kind == "k":
            groups[gidx].append((k_hbm.at[hs], kb.at[hs]))
            for h in range(h0, h0 + n): need_k[h] = gidx
        else:
            groups[gidx].append((v_hbm.at[hs], vb.at[hs]))
            for h in range(h0, h0 + n): need_v[h] = gidx
    h0 = 0
    for r, n in enumerate(ramp):
        if r == 0 and split0:
            assert n == 1
            groups.append([]); add(0, "k", 0, 1); add(0, "q", 0, 1, 0, split0)
            groups.append([]); add(1, "v", 0, 1); add(1, "q", 0, 1, split0, M)
        else:
            groups.append([]); gi = len(groups) - 1
            add(gi, "k", h0, n); add(gi, "q", h0, n); add(gi, "v", h0, n)
        h0 += n
    assert h0 == nh
    def rcopies(gi):
        return [pltpu.make_async_copy(s, d, rsem.at[gi]) for s, d in groups[gi]]
    def grp_copies(gi, s):
        src = pl.ds(gi * nh, nh)
        dst = pl.ds(s * nh, nh)
        return [pltpu.make_async_copy(k_hbm.at[src], kb.at[dst], isem.at[s]),
                pltpu.make_async_copy(q_hbm.at[src], qb.at[dst], isem.at[s]),
                pltpu.make_async_copy(v_hbm.at[src], vb.at[dst], isem.at[s])]
    def grp_out(gi):
        sl = pl.ds(gi * nh, nh)
        return pltpu.make_async_copy(ob.at[sl], o_hbm.at[sl], osem.at[gi])

    issue = [rcopies(gi) for gi in range(len(groups))] + [grp_copies(gi, gi % ns) for gi in range(1, ns)]
    state = dict(issued=0, waited=-1, pending=0)
    def issue_next():
        if state["issued"] < len(issue):
            for c in issue[state["issued"]]:
                c.start()
            state["issued"] += 1
    for _ in range(lead):
        issue_next()
    def ensure(g):
        while state["waited"] < g:
            state["waited"] += 1
            assert state["issued"] > state["waited"]
            for c in rcopies(state["waited"]):
                c.wait()
            state["pending"] += 1
    def after_mxu():
        while state["pending"]:
            issue_next(); state["pending"] -= 1
    units = []
    for h in range(nh):
        u_r = ur0 if h == 0 else ur
        units += [(h, r0, r0 + u_r) for r0 in range(0, M, u_r)]
    def bq(u):
        h, r0, r1 = units[u]
        ensure(max(need_k[h], max(need_q[(h, r)] for r in range(r0, r1, 8))))
    def bp(u):
        ensure(need_v[units[u][0]])
    def put(u, h, r0, r1, o):
        ob[h, r0:r1] = o.astype(ob.dtype)
    pipeline(units, lambda h, r0, r1: qb[h, r0:r1], lambda h: kb[h], lambda h: vb[h], put, scale, recip, bq, bp, after_mxu)
    while state["issued"] < len(issue):
        issue_next()
    grp_out(0).start()

    lunits = [(h, r0, r0 + ur) for h in range(nh) for r0 in range(0, M, ur)]
    if tail < ur:
        h, r0, r1 = lunits.pop()
        lunits += [(h, r, r + tail) for r in range(r0, r1, tail)]
    def body(gi, carry):
        s = gi % ns
        for c in grp_copies(gi, s):
            c.wait()
        def bp(u):
            if u == 0:
                @pl.when(gi + ns - 1 < ng)
                def _():
                    for c in grp_copies(gi + ns - 1, (gi + ns - 1) % ns):
                        c.start()
        def put(u, h, r0, r1, o):
            g = gi * nh + h
            ob[g, r0:r1] = o.astype(ob.dtype)
            if h == nh - 1:
                pltpu.make_async_copy(ob.at[g, r0:r1], o_hbm.at[g, r0:r1], osem.at[gi]).start()
            elif r1 == M:
                pltpu.make_async_copy(ob.at[g], o_hbm.at[g], osem.at[gi]).start()
        b0 = s * nh
        pipeline(lunits, lambda h, r0, r1: qb[b0 + h, r0:r1], lambda h: kb[b0 + h], lambda h: vb[b0 + h], put, scale, recip, None, bp)
        return carry
    lax.fori_loop(1, ng, body, 0)

    for gi in range(ng):
        grp_out(gi).wait()


@jax.jit
def pallas_standalone__gqa_softmax__near_ridge_kernel(
    q: jax.Array,
    k: jax.Array,
    v: jax.Array,
):
    B, Hq, Sq, D = q.shape
    Hkv, Sk = k.shape[1], k.shape[2]
    rep = Hq // Hkv
    G = B * Hkv
    M = rep * Sq
    nh, ns, ramp = 8, 3, (1, 1, 2, 4)
    ng = G // nh
    q3 = q.reshape(G, M, D)
    k3 = k.reshape(G, Sk, D)
    v3 = v.reshape(G, Sk, D)
    scale = D ** -0.5
    out = pl.pallas_call(
        functools.partial(_kernel, scale=scale, nh=nh, G=G, M=M, ramp=ramp, recip="nr", ns=ns,
                          ur=512, ur0=256, split0=512, tail=256, lead=3),
        in_specs=[pl.BlockSpec(memory_space=pl.ANY)] * 3,
        out_specs=pl.BlockSpec(memory_space=pl.ANY),
        out_shape=jax.ShapeDtypeStruct((G, M, D), q.dtype),
        scratch_shapes=[
            pltpu.VMEM((ns * nh, M, D), q.dtype),
            pltpu.VMEM((ns * nh, Sk, D), q.dtype),
            pltpu.VMEM((ns * nh, Sk, D), q.dtype),
            pltpu.VMEM((G, M, D), q.dtype),
            pltpu.SemaphoreType.DMA((len(ramp) + 1,)),
            pltpu.SemaphoreType.DMA((ns,)),
            pltpu.SemaphoreType.DMA((ng,)),
        ],
        compiler_params=pltpu.CompilerParams(
            vmem_limit_bytes=100 * 1024 * 1024,
            disable_bounds_checks=True,
            disable_semaphore_checks=True,
        ),
    )(q3, k3, v3)
    return out.reshape(B, Hq, Sq, D)
```

```python
import functools
import math

import jax
import jax.numpy as jnp
from jax import lax
import jax.experimental.pallas as pl
import jax.experimental.pallas.tpu as pltpu

_LANES = 128


def _qk(q, k):
    return lax.dot_general(q, k, (((1,), (1,)), ((), ())),
                           preferred_element_type=jnp.float32)


def _softmax_parts(s, scale):
    m = jnp.max(s, axis=-1, keepdims=True)
    p = jnp.exp2((s - m) * (scale * math.log2(math.e)))
    l = jnp.sum(p, axis=-1, keepdims=True)
    r = pl.reciprocal(l, approx=True)
    r = r * (2.0 - l * r)
    p_last = jnp.minimum(p[:, -_LANES:], l)
    p = jnp.concatenate([p[:, :-_LANES], p_last], axis=1).astype(jnp.bfloat16)
    return p, r


def _pipeline(units, get_q, get_k, get_v, put, scale,
              before_qk=None, before_pv=None, after_mxu=None):
    n = len(units)

    def do_qk(u):
        if before_qk is not None:
            before_qk(u)
        h, r0, r1 = units[u]
        s = _qk(get_q(h, r0, r1), get_k(h))
        if after_mxu is not None:
            after_mxu()
        return s

    s_next = do_qk(0)
    for u in range(n):
        s = s_next
        if u + 1 < n:
            s_next = do_qk(u + 1)
        p, r = _softmax_parts(s, scale)
        if before_pv is not None:
            before_pv(u)
        h, r0, r1 = units[u]
        o = jnp.dot(p, get_v(h), preferred_element_type=jnp.float32) * r
        if after_mxu is not None:
            after_mxu()
        put(u, h, r0, r1, o)


def _make_units(spec):
    units = []
    for h, rows in enumerate(spec):
        r0 = 0
        for r in rows:
            units.append((h, r0, r0 + r))
            r0 += r
    return units


def _attn_kernel(q_hbm, k_hbm, v_hbm, o_hbm, qb, kb, vb, ob, rsem, isem, osem,
                 *, scale, nh, G, M, ns, ramp, lead, ochunk):
    ng = G // nh
    half, quarter = M // 2, M // 4

    groups = [
        [(k_hbm.at[0], kb.at[0]), (q_hbm.at[0, 0:half], qb.at[0, 0:half])],
        [(v_hbm.at[0], vb.at[0]), (q_hbm.at[0, half:M], qb.at[0, half:M])],
    ]
    group_of_head = {}
    ramp_spec = [[quarter] * 4]
    h0 = 1
    for n in ramp:
        hs = pl.ds(h0, n)
        groups.append([(k_hbm.at[hs], kb.at[hs]), (q_hbm.at[hs], qb.at[hs]),
                       (v_hbm.at[hs], vb.at[hs])])
        for h in range(h0, h0 + n):
            group_of_head[h] = len(groups) - 1
            last_before_wait = h == h0 + n - 1 and h != nh - 1
            ramp_spec.append([half, quarter, quarter] if last_before_wait
                             else [half, half])
        h0 += n
    assert h0 == nh

    def ramp_copies(g):
        return [pltpu.make_async_copy(s, d, rsem.at[g]) for s, d in groups[g]]

    def group_copies(gi, slot):
        src = pl.ds(gi * nh, nh)
        dst = pl.ds(slot * nh, nh)
        return [pltpu.make_async_copy(k_hbm.at[src], kb.at[dst], isem.at[slot]),
                pltpu.make_async_copy(q_hbm.at[src], qb.at[dst], isem.at[slot]),
                pltpu.make_async_copy(v_hbm.at[src], vb.at[dst], isem.at[slot])]

    def group_out(gi):
        sl = pl.ds(gi * nh, nh)
        return pltpu.make_async_copy(ob.at[sl], o_hbm.at[sl], osem.at[gi])

    issue = [ramp_copies(g) for g in range(len(groups))]
    issue += [group_copies(gi, gi) for gi in range(1, ns)]
    state = dict(issued=0, waited=-1, pending=0)

    def issue_next():
        if state["issued"] < len(issue):
            for c in issue[state["issued"]]:
                c.start()
            state["issued"] += 1

    def ensure(g):
        while state["waited"] < g:
            state["waited"] += 1
            assert state["issued"] > state["waited"]
            for c in ramp_copies(state["waited"]):
                c.wait()
            state["pending"] += 1

    def after_mxu():
        while state["pending"]:
            issue_next()
            state["pending"] -= 1

    for _ in range(lead):
        issue_next()

    units = _make_units(ramp_spec)

    def need_qk(u):
        h, _, r1 = units[u]
        if h == 0:
            return 0 if r1 <= half else 1
        return group_of_head[h]

    def ramp_before_pv(u):
        h = units[u][0]
        need = 1 if h == 0 else group_of_head[h]
        if u + 2 < len(units):
            need = max(need, need_qk(u + 2))
        ensure(need)

    def ramp_put(u, h, r0, r1, o):
        ob[h, r0:r1] = o.astype(ob.dtype)

    _pipeline(units, lambda h, r0, r1: qb[h, r0:r1], lambda h: kb[h],
              lambda h: vb[h], ramp_put, scale,
              lambda u: ensure(need_qk(u)), ramp_before_pv, after_mxu)
    while state["issued"] < len(issue):
        issue_next()

    lunits = _make_units([[M]] * (nh - 1) + [[half, quarter, quarter]])

    def body(gi, slot):
        for c in group_copies(gi, slot):
            c.wait()
        slot_prev = jnp.where(slot == 0, ns - 1, slot - 1)
        slot_next = jnp.where(slot == ns - 1, 0, slot + 1)

        def before_pv(u):
            if u == 0:
                @pl.when(gi + ns - 1 < ng)
                def _():
                    for c in group_copies(gi + ns - 1, slot_prev):
                        c.start()

                @pl.when(gi == ng - 2)
                def _():
                    group_out(0).start()

        def put(u, h, r0, r1, o):
            g = gi * nh + h
            o = o.astype(ob.dtype)
            step = ochunk if h == nh - 1 else r1 - r0
            for a in range(r0, r1, step):
                ob[g, a:a + step] = o[a - r0:a - r0 + step]
                pltpu.make_async_copy(ob.at[g, a:a + step],
                                      o_hbm.at[g, a:a + step],
                                      osem.at[gi]).start()

        b0 = slot * nh
        _pipeline(lunits, lambda h, r0, r1: qb[b0 + h, r0:r1],
                  lambda h: kb[b0 + h], lambda h: vb[b0 + h], put, scale,
                  None, before_pv)
        return slot_next

    lax.fori_loop(1, ng, body, jnp.int32(1))

    for gi in range(ng):
        group_out(gi).wait()


@jax.jit
def pallas_standalone__gqa_softmax__near_ridge_kernel(
    q: jax.Array,
    k: jax.Array,
    v: jax.Array,
):
    B, Hq, Sq, D = q.shape
    Hkv, Sk = k.shape[1], k.shape[2]
    rep = Hq // Hkv
    G = B * Hkv
    M = rep * Sq
    nh, ns, ramp = 8, 3, (1, 2, 4)
    assert G % nh == 0 and G // nh >= ns
    q3 = q.reshape(G, M, D)
    k3 = k.reshape(G, Sk, D)
    v3 = v.reshape(G, Sk, D)
    out = pl.pallas_call(
        functools.partial(_attn_kernel, scale=D ** -0.5, nh=nh, G=G, M=M,
                          ns=ns, ramp=ramp, lead=3, ochunk=64),
        in_specs=[pl.BlockSpec(memory_space=pl.ANY)] * 3,
        out_specs=pl.BlockSpec(memory_space=pl.ANY),
        out_shape=jax.ShapeDtypeStruct((G, M, D), q.dtype),
        scratch_shapes=[
            pltpu.VMEM((ns * nh, M, D), q.dtype),
            pltpu.VMEM((ns * nh, Sk, D), k.dtype),
            pltpu.VMEM((ns * nh, Sk, D), v.dtype),
            pltpu.VMEM((G, M, D), q.dtype),
            pltpu.SemaphoreType.DMA((len(ramp) + 2,)),
            pltpu.SemaphoreType.DMA((ns,)),
            pltpu.SemaphoreType.DMA((G // nh,)),
        ],
        compiler_params=pltpu.CompilerParams(
            vmem_limit_bytes=100 * 1024 * 1024,
            disable_bounds_checks=True,
            disable_semaphore_checks=True,
        ),
    )(q3, k3, v3)
    return out.reshape(B, Hq, Sq, D)
```

```python
import functools
import math

import jax
import jax.numpy as jnp
from jax import lax
import jax.experimental.pallas as pl
import jax.experimental.pallas.tpu as pltpu

_LANES = 128


def _qk(q, k):
    return lax.dot_general(q, k, (((1,), (1,)), ((), ())),
                           preferred_element_type=jnp.float32)


def _softmax_parts(s, scale):
    tiles = [s[:, j:j + _LANES] for j in range(0, s.shape[1], _LANES)]
    while len(tiles) > 1:
        tiles = [jnp.maximum(*tiles[j:j + 2]) if j + 1 < len(tiles) else tiles[j]
                 for j in range(0, len(tiles), 2)]
    m = jnp.max(tiles[0], axis=-1, keepdims=True)
    p = jnp.exp2((s - m) * (scale * math.log2(math.e)))
    l = jnp.sum(p, axis=-1, keepdims=True)
    r = pl.reciprocal(l, approx=True)
    r = r * (2.0 - l * r)
    p_last = jnp.minimum(p[:, -_LANES:], l)
    p = jnp.concatenate([p[:, :-_LANES], p_last], axis=1).astype(jnp.bfloat16)
    return p, r


def _pipeline(units, scores, get_v, put, scale,
              before_qk=None, before_pv=None, after_mxu=None):
    n = len(units)

    def do_qk(u):
        if before_qk is not None:
            before_qk(u)
        s = scores(u, *units[u])
        if after_mxu is not None:
            after_mxu()
        return s

    s_next = do_qk(0)
    for u in range(n):
        s = s_next
        if u + 1 < n:
            s_next = do_qk(u + 1)
        p, r = _softmax_parts(s, scale)
        if before_pv is not None:
            before_pv(u)
        h, r0, r1 = units[u]
        o = jnp.dot(p, get_v(h), preferred_element_type=jnp.float32) * r
        if after_mxu is not None:
            after_mxu()
        put(u, h, r0, r1, o)


def _make_units(spec):
    units = []
    for h, rows in enumerate(spec):
        r0 = 0
        for r in rows:
            units.append((h, r0, r0 + r))
            r0 += r
    return units


def _attn_kernel(q_hbm, k_hbm, v_hbm, o_hbm, qb, kb, vb, ob, k0b, ktb,
                 rsem, isem, osem, *, scale, nh, G, M, ns, ramp, lead, ochunk):
    ng = G // nh
    half, quarter = M // 2, M // 4
    kh = k0b.shape[1]

    groups = [
        [(k_hbm.at[0], kb.at[0]), (q_hbm.at[0, 0:half], qb.at[0, 0:half])],
        [(v_hbm.at[0], vb.at[0]), (q_hbm.at[0, half:M], qb.at[0, half:M])],
    ]
    group_of_head = {}
    ramp_spec = [[quarter] * 4]
    h0 = 1
    for n in ramp:
        hs = pl.ds(h0, n)
        groups.append([(k_hbm.at[hs], kb.at[hs]), (q_hbm.at[hs], qb.at[hs]),
                       (v_hbm.at[hs], vb.at[hs])])
        for h in range(h0, h0 + n):
            group_of_head[h] = len(groups) - 1
            last_before_wait = h == h0 + n - 1 and h != nh - 1
            ramp_spec.append([half, quarter, quarter] if last_before_wait
                             else [half, half])
        h0 += n
    assert h0 == nh
    groups[-1].append((k_hbm.at[nh, 0:kh], k0b.at[0]))

    def ramp_copies(g):
        return [pltpu.make_async_copy(s, d, rsem.at[g]) for s, d in groups[g]]

    def group_copies(gi, slot):
        src = pl.ds(gi * nh, nh)
        dst = pl.ds(slot * nh, nh)
        nxt = jnp.minimum(gi + 1, ng - 1) * nh
        sem = isem.at[slot]
        return [pltpu.make_async_copy(k_hbm.at[nxt, 0:kh], k0b.at[slot], sem),
                pltpu.make_async_copy(k_hbm.at[src], kb.at[dst], sem),
                pltpu.make_async_copy(q_hbm.at[src], qb.at[dst], sem),
                pltpu.make_async_copy(v_hbm.at[src], vb.at[dst], sem)]

    def group_out(gi):
        sl = pl.ds(gi * nh, nh)
        return pltpu.make_async_copy(ob.at[sl], o_hbm.at[sl], osem.at[gi])

    issue = [ramp_copies(g) for g in range(len(groups))]
    issue += [group_copies(gi, gi) for gi in range(1, ns)]
    state = dict(issued=0, waited=-1, pending=0)

    def issue_next():
        if state["issued"] < len(issue):
            for c in issue[state["issued"]]:
                c.start()
            state["issued"] += 1

    def ensure(g):
        while state["waited"] < g:
            state["waited"] += 1
            assert state["issued"] > state["waited"]
            for c in ramp_copies(state["waited"]):
                c.wait()
            state["pending"] += 1

    def after_mxu():
        while state["pending"]:
            issue_next()
            state["pending"] -= 1

    for _ in range(lead):
        issue_next()

    units = _make_units(ramp_spec)

    def need_qk(u):
        h, _, r1 = units[u]
        if h == 0:
            return 0 if r1 <= half else 1
        return group_of_head[h]

    def ramp_before_pv(u):
        h = units[u][0]
        need = 1 if h == 0 else group_of_head[h]
        if u + 2 < len(units):
            need = max(need, need_qk(u + 2))
        ensure(need)

    def ramp_put(u, h, r0, r1, o):
        ob[h, r0:r1] = o.astype(ob.dtype)
        if u == len(units) - 4:
            assert state["waited"] == len(groups) - 1
            ktb[...] = k0b[0].T

    _pipeline(units, lambda u, h, r0, r1: _qk(qb[h, r0:r1], kb[h]),
              lambda h: vb[h], ramp_put, scale,
              lambda u: ensure(need_qk(u)), ramp_before_pv, after_mxu)
    while state["issued"] < len(issue):
        issue_next()

    lunits = _make_units([[M]] * (nh - 1) + [[half, quarter, quarter]])

    def body(gi, slot):
        for c in group_copies(gi, slot):
            c.wait()
        slot_prev = jnp.where(slot == 0, ns - 1, slot - 1)
        slot_next = jnp.where(slot == ns - 1, 0, slot + 1)
        b0 = slot * nh

        def scores(u, h, r0, r1):
            q = qb[b0 + h, r0:r1]
            if u > 0:
                return _qk(q, kb[b0 + h])
            s_lo = jnp.dot(q, ktb[...], preferred_element_type=jnp.float32)
            return jnp.concatenate([s_lo, _qk(q, kb[b0, kh:])], axis=1)

        def before_pv(u):
            if u == 0:
                @pl.when(gi + ns - 1 < ng)
                def _():
                    for c in group_copies(gi + ns - 1, slot_prev):
                        c.start()

                @pl.when(gi == ng - 2)
                def _():
                    group_out(0).start()

        def put(u, h, r0, r1, o):
            g = gi * nh + h
            o = o.astype(ob.dtype)
            step = ochunk if h == nh - 1 else r1 - r0
            for a in range(r0, r1, step):
                ob[g, a:a + step] = o[a - r0:a - r0 + step]
                pltpu.make_async_copy(ob.at[g, a:a + step],
                                      o_hbm.at[g, a:a + step],
                                      osem.at[gi]).start()
            if u == 3:
                ktb[...] = k0b[slot].T

        _pipeline(lunits, scores, lambda h: vb[b0 + h], put, scale,
                  None, before_pv)
        return slot_next

    lax.fori_loop(1, ng, body, jnp.int32(1))

    for gi in range(ng):
        group_out(gi).wait()


@jax.jit
def pallas_standalone__gqa_softmax__near_ridge_kernel(
    q: jax.Array,
    k: jax.Array,
    v: jax.Array,
):
    B, Hq, Sq, D = q.shape
    Hkv, Sk = k.shape[1], k.shape[2]
    rep = Hq // Hkv
    G = B * Hkv
    M = rep * Sq
    nh, ns, ramp = 8, 3, (1, 2, 4)
    assert G % nh == 0 and G // nh >= ns
    q3 = q.reshape(G, M, D)
    k3 = k.reshape(G, Sk, D)
    v3 = v.reshape(G, Sk, D)
    out = pl.pallas_call(
        functools.partial(_attn_kernel, scale=D ** -0.5, nh=nh, G=G, M=M,
                          ns=ns, ramp=ramp, lead=3, ochunk=64),
        in_specs=[pl.BlockSpec(memory_space=pl.ANY)] * 3,
        out_specs=pl.BlockSpec(memory_space=pl.ANY),
        out_shape=jax.ShapeDtypeStruct((G, M, D), q.dtype),
        scratch_shapes=[
            pltpu.VMEM((ns * nh, M, D), q.dtype),
            pltpu.VMEM((ns * nh, Sk, D), k.dtype),
            pltpu.VMEM((ns * nh, Sk, D), v.dtype),
            pltpu.VMEM((G, M, D), q.dtype),
            pltpu.VMEM((ns, Sk // 2, D), k.dtype),
            pltpu.VMEM((D, Sk // 2), k.dtype),
            pltpu.SemaphoreType.DMA((len(ramp) + 2,)),
            pltpu.SemaphoreType.DMA((ns,)),
            pltpu.SemaphoreType.DMA((G // nh,)),
        ],
        compiler_params=pltpu.CompilerParams(
            vmem_limit_bytes=100 * 1024 * 1024,
            disable_bounds_checks=True,
            disable_semaphore_checks=True,
        ),
    )(q3, k3, v3)
    return out.reshape(B, Hq, Sq, D)
```
